```python
import os as _os
_os.environ.setdefault("JAX_PLATFORMS", "cpu")
import jax
import jax.numpy as jnp

def _softmax(x, axis=-1):
    return jax.nn.softmax(x, axis=axis)
def _gelu(x):
    return jax.nn.gelu(x, approximate=True)
def _silu(x):
    return jax.nn.silu(x)
def _sigmoid(x):
    return jax.nn.sigmoid(x)
def _layernorm(x, axis=-1, eps=1e-5):
    m = jnp.mean(x, axis=axis, keepdims=True)
    v = jnp.var(x, axis=axis, keepdims=True)
    return (x - m) / jnp.sqrt(v + eps)
def _scatter_add(tgt, idx, src, axis=0):
    return tgt.at[idx].add(src)
def _segment_sum(src, seg, n):
    return jax.ops.segment_sum(src, seg, n)
class _Rng:
    def __init__(self, key):
        self._k = key
    def _next(self):
        self._k, sub = jax.random.split(self._k)
        return sub
    def normal(self, shape):
        return jax.random.normal(self._next(), shape, dtype=jnp.bfloat16)
    def randint(self, lo, hi, shape):
        return jax.random.randint(self._next(), shape, lo, hi, dtype=jnp.int32)
    def uniform(self, shape, lo=0.0, hi=1.0):
        return jax.random.uniform(self._next(), shape, jnp.bfloat16, lo, hi)
    def permutation(self, n):
        return jax.random.permutation(self._next(), n)


kernel_name = 'concat_heads__mha_block_cached__mha_block_cached__near_ridge'

def setup_inputs():
    _rng = _Rng(jax.random.key(int.from_bytes(__import__("os").urandom(4), "little")))
    _w = (lambda a: (lambda t: t.astype(jnp.bfloat16) if jnp.issubdtype(t.dtype, jnp.floating) else t)(jnp.asarray(a)))
    def _A_setup():
        B, Sq, D = 8, 160, 512
        H, Sk, Dh = 32, 512, 128
        return {
            "x": _w((lambda *s: _rng.normal(s) * 0.8)(B, Sq, D)),
            "k_cache": _w((lambda *s: _rng.normal(s) * 0.8)(B, H, Sk, Dh)),
            "v_cache": _w((lambda *s: _rng.normal(s) * 0.05)(B, H, Sk, Dh)),
            "wq": _w((lambda *s: _rng.normal(s) * 0.8)(D, H * Dh) * (D ** -0.5)),
            "wo": _w((lambda *s: _rng.normal(s) * 0.05)(H * Dh, D) * ((H * Dh) ** -0.5)),
        }
    _A_in = _A_setup()

    def _B_setup():
        B, Sq, D = 8, 160, 512
        H, Sk, Dh = 32, 512, 128
        return {
            "x": _w((lambda *s: _rng.normal(s) * 0.8)(B, Sq, D)),
            "k_cache": _w((lambda *s: _rng.normal(s) * 0.8)(B, H, Sk, Dh)),
            "v_cache": _w((lambda *s: _rng.normal(s) * 0.05)(B, H, Sk, Dh)),
            "wq": _w((lambda *s: _rng.normal(s) * 0.8)(D, H * Dh) * (D ** -0.5)),
            "wo": _w((lambda *s: _rng.normal(s) * 0.05)(H * Dh, D) * ((H * Dh) ** -0.5)),
        }
    _B_in = _B_setup()

    return {
        "A_x": _A_in["x"],
        "A_k_cache": _A_in["k_cache"],
        "A_v_cache": _A_in["v_cache"],
        "A_wq": _A_in["wq"],
        "A_wo": _A_in["wo"],
        "B_x": _B_in["x"],
        "B_k_cache": _B_in["k_cache"],
        "B_v_cache": _B_in["v_cache"],
        "B_wq": _B_in["wq"],
        "B_wo": _B_in["wo"],
    }

def reference(A_x, A_k_cache, A_v_cache, A_wq, A_wo, B_x, B_k_cache, B_v_cache, B_wq, B_wo):
    def _A_ref(x, k_cache, v_cache, wq, wo):
        B, Sq, D = x.shape
        H, Dh = 32, 128
        q = (lambda x, *d: x.transpose(*d))((x @ wq).reshape(B, Sq, H, Dh), 0, 2, 1, 3)
        scores = jnp.einsum("bhqd,bhkd->bhqk", q, k_cache) * (Dh ** -0.5)
        p = _softmax(scores, axis=-1)
        o = jnp.einsum("bhqk,bhkd->bhqd", p, v_cache)
        return (lambda x, *d: x.transpose(*d))(o, 0, 2, 1, 3).reshape(B, Sq, H * Dh) @ wo

    def _B_ref(x, k_cache, v_cache, wq, wo):
        B, Sq, D = x.shape
        H, Dh = 32, 128
        q = (lambda x, *d: x.transpose(*d))((x @ wq).reshape(B, Sq, H, Dh), 0, 2, 1, 3)
        scores = jnp.einsum("bhqd,bhkd->bhqk", q, k_cache) * (Dh ** -0.5)
        p = _softmax(scores, axis=-1)
        o = jnp.einsum("bhqk,bhkd->bhqd", p, v_cache)
        return (lambda x, *d: x.transpose(*d))(o, 0, 2, 1, 3).reshape(B, Sq, H * Dh) @ wo

    a = _A_ref(A_x, A_k_cache, A_v_cache, A_wq, A_wo)
    b = _B_ref(B_x, B_k_cache, B_v_cache, B_wq, B_wo)
    return jnp.concatenate([a, b], axis=-1)
```

```python
import functools
import jax
import jax.numpy as jnp
import numpy as np
import jax.experimental.pallas as pl
import jax.experimental.pallas.tpu as pltpu

B, SQ, D = 8, 160, 512
H, SK, DH = 32, 512, 128
M = B * SQ
LOG2E = float(np.log2(np.e))
SCALE = float(DH ** -0.5)


def _kernel(ax, ak, av, awq, awo, bx, bk, bv, bwq, bwo, out_ref, acc_a, acc_b):
    g = pl.program_id(0)

    @pl.when(g == 0)
    def _():
        acc_a[...] = jnp.zeros_like(acc_a)
        acc_b[...] = jnp.zeros_like(acc_b)

    items = [(ax, ak, av, awq, awo, acc_a, b) for b in range(B)] + [(bx, bk, bv, bwq, bwo, acc_b, b) for b in range(B)]
    n = len(items)
    q, s, p, l, o = {}, {}, {}, {}, {}

    def QP(i):
        x, k, v, wq, wo, acc, b = items[i]
        r = jnp.dot(x[b * SQ:(b + 1) * SQ, :], wq[...], preferred_element_type=jnp.float32)
        q[i] = (r * (SCALE * LOG2E)).astype(jnp.bfloat16)

    def QK(i):
        x, k, v, wq, wo, acc, b = items[i]
        s[i] = jax.lax.dot_general(q.pop(i), k[b, 0], (((1,), (1,)), ((), ())), preferred_element_type=jnp.float32)

    def SM(i):
        si = s.pop(i)
        m = jnp.max(si, axis=-1, keepdims=True)
        e = jnp.exp2(si - m)
        l[i] = jnp.sum(e, axis=-1, keepdims=True)
        p[i] = e.astype(jnp.bfloat16)

    def PV(i):
        x, k, v, wq, wo, acc, b = items[i]
        r = jnp.dot(p.pop(i), v[b, 0], preferred_element_type=jnp.float32)
        o[i] = (r * pl.reciprocal(l.pop(i), approx=False)).astype(jnp.bfloat16)

    def OP(i):
        x, k, v, wq, wo, acc, b = items[i]
        acc[b * SQ:(b + 1) * SQ, :] += jnp.dot(o.pop(i), wo[...], preferred_element_type=jnp.float32)

    QP(0); QP(1); QK(0)
    for i in range(n):
        if i + 1 < n: QK(i + 1)
        if i + 2 < n: QP(i + 2)
        SM(i)
        PV(i)
        if i >= 1: OP(i - 1)
    OP(n - 1)

    @pl.when(g == pl.num_programs(0) - 1)
    def _():
        out_ref[:, 0:D] = acc_a[...].astype(out_ref.dtype)
        out_ref[:, D:2 * D] = acc_b[...].astype(out_ref.dtype)


@jax.jit
def pallas_concat_heads__mha_block_cached__mha_block_cached__near_ridge_kernel(
    A_x, A_k_cache, A_v_cache, A_wq, A_wo, B_x, B_k_cache, B_v_cache, B_wq, B_wo):
    specs = [
        pl.BlockSpec((M, D), lambda g: (0, 0)),
        pl.BlockSpec((B, 1, SK, DH), lambda g: (0, g, 0, 0)),
        pl.BlockSpec((B, 1, SK, DH), lambda g: (0, g, 0, 0)),
        pl.BlockSpec((D, DH), lambda g: (0, g)),
        pl.BlockSpec((DH, D), lambda g: (g, 0)),
    ]
    out = pl.pallas_call(
        _kernel,
        grid=(H,),
        in_specs=specs + specs,
        out_specs=pl.BlockSpec((M, 2 * D), lambda g: (0, 0)),
        out_shape=jax.ShapeDtypeStruct((M, 2 * D), jnp.bfloat16),
        scratch_shapes=[pltpu.VMEM((M, D), jnp.float32), pltpu.VMEM((M, D), jnp.float32)],
        compiler_params=pltpu.CompilerParams(
            dimension_semantics=("arbitrary",),
            vmem_limit_bytes=100 * 1024 * 1024),
    )(A_x.reshape(M, D), A_k_cache, A_v_cache, A_wq, A_wo,
      B_x.reshape(M, D), B_k_cache, B_v_cache, B_wq, B_wo)
    return out.reshape(B, SQ, 2 * D)
```

```python
import contextlib
import os
import jax
import jax.numpy as jnp
import numpy as np
import jax.experimental.pallas as pl
import jax.experimental.pallas.tpu as pltpu

B, SQ, D = 8, 160, 512
H, SK, DH = 32, 512, 128
M = B * SQ
QSCALE = float(DH ** -0.5) * float(np.log2(np.e))

def _env(n, d):
    return os.environ.get(n, d)

G = int(_env("G", 4))
NS = int(_env("NS", 4))
U = G * B
NC = H // G
GW = G * DH
RA = -(-M // ((NC - 1) * 16)) * 16
XR = [int(v) for v in _env("XR", "1,2,2,3").split(",")]
WG = [int(v) for v in _env("WG", "4,8,10,10").split(",")]
PRESTAGE = [int(float(v) * 2**20) for v in _env("PRESTAGE", "14,9,9").split(",")]
SCOPES = [v for v in _env("SCOPES", "").split(",") if v]
scope = lambda n: jax.named_scope(n) if (n in SCOPES or "1" in SCOPES) else contextlib.nullcontext()


def _kernel(ax, ak, av, awq, awo, bx, bk, bv, bwq, bwo, out,
            xb, kb, vb, wqa, wqb, wob, qb, acc, ob, s_scr, o_scr,
            xsem, ksem, vsem, wqasem, wqsem, wosem, osem):
    xs, ks, vs, wos = (ax, bx), (ak, bk), (av, bv), (awo, bwo)

    def cp_x(br, r0, n, i):
        return pltpu.make_async_copy(xs[br].at[pl.ds(r0, n)], xb.at[br, pl.ds(r0, n)], xsem.at[i])

    def cp_k(br, c, slot):
        return pltpu.make_async_copy(ks[br].at[:, pl.ds(c * G, G)], kb.at[slot], ksem.at[slot])

    def cp_v(br, c, slot):
        return pltpu.make_async_copy(vs[br].at[:, pl.ds(c * G, G)], vb.at[slot], vsem.at[slot])

    def cp_wqa(h0, nh, i):
        return pltpu.make_async_copy(awq.at[:, h0 * DH:(h0 + nh) * DH], wqa.at[:, h0 * DH:(h0 + nh) * DH], wqasem.at[i])

    def cp_wq(c):
        return pltpu.make_async_copy(bwq.at[:, pl.ds(pl.multiple_of(c * GW, GW), GW)], wqb.at[c], wqsem.at[c])

    def cp_wo(br, c):
        return pltpu.make_async_copy(wos[br].at[pl.ds(pl.multiple_of(c * GW, GW), GW), :],
                                     wob.at[br * NC + c], wosem.at[br * NC + c])

    def start_chunk(br, c, slot):
        cp_k(br, c, slot).start()
        cp_v(br, c, slot).start()
        cp_wo(br, c).start()
        if br == 0:
            cp_wq(c).start()

    def wait(dst, sem):
        pltpu.make_async_copy(dst, dst, sem).wait()

    def rows(b):
        return slice(b * SQ, (b + 1) * SQ)

    def cols(h):
        return slice(h * DH, (h + 1) * DH)

    def proj_q(x, w):
        r = jnp.dot(x, w, preferred_element_type=jnp.float32)
        return (r * QSCALE).astype(jnp.bfloat16)

    def QK(g, t, slot):
        h, b = t // B, t % B
        return jax.lax.dot_general(qb[g, rows(b), cols(h)], kb[slot, b, h], (((1,), (1,)), ((), ())),
                                   preferred_element_type=jnp.float32)

    def SM(s):
        m = jnp.max(s, axis=-1, keepdims=True)
        e = jnp.exp2(s - m)
        return e.astype(jnp.bfloat16), jnp.sum(e, axis=-1, keepdims=True)

    def PV(p, l, t, slot):
        h, b = t // B, t % B
        r = jnp.dot(p, vb[slot, b, h], preferred_element_type=jnp.float32)
        return (r * pltpu.reciprocal(l, approx=False, full_range=False)).astype(jnp.bfloat16)

    def OP(o, br, g, t, final=False):
        h, b = t // B, t % B
        r = acc[br, rows(b), :] + jnp.dot(o, wob[g, cols(h), :], preferred_element_type=jnp.float32)
        if final:
            ob[1, rows(b), :] = r.astype(jnp.bfloat16)
        else:
            acc[br, rows(b), :] = r

    xr, wg = [], []
    for n in XR:
        xr.append((sum(v[1] for v in xr), n * SQ))
    for n in WG:
        wg.append((sum(v[1] for v in wg), n))

    def qp_a(r0, n, h0, nh):
        r = proj_q(xb[0, r0:r0 + n, :], wqa[:, h0 * DH:(h0 + nh) * DH])
        for h in range(h0, h0 + nh):
            qb[h // G, r0:r0 + n, cols(h % G)] = r[:, cols(h - h0)]

    KVB, WB, XB = B * G * SK * DH * 2, D * GW * 2, M * D * 2
    pre = [(cp_k(0, 0, 0), KVB), (cp_v(0, 0, 0), KVB), (cp_wo(0, 0), WB), (cp_wq(0), WB), (cp_x(1, 0, M, len(xr)), XB)]
    for g in range(1, NS):
        pre += [(cp_k(0, g, g), KVB), (cp_v(0, g, g), KVB), (cp_wo(0, g), WB), (cp_wq(g), WB)]
    stages, cur, lim = [[]], 0, list(PRESTAGE)
    for cpy, nb in pre:
        if lim and cur >= lim[0]:
            stages.append([]); cur = 0; lim.pop(0)
        stages[-1].append(cpy); cur += nb

    def pre_stage():
        if stages:
            for cpy in stages.pop(0):
                cpy.start()

    cp_x(0, *xr[0], 0).start()
    cp_wqa(*wg[0], 0).start()
    cp_x(0, *xr[1], 1).start()
    acc[...] = jnp.zeros_like(acc)
    o_scr[...] = jnp.zeros_like(o_scr)
    queue = [[cp_x(0, *xr[i], i)] for i in range(2, len(xr))]
    queue += [[cp_wqa(*wg[1], 1)], [cp_wqa(*wg[i], i) for i in range(2, len(wg))]]
    for i in range(len(xr)):
        cp_x(0, *xr[i], i).wait()
        if i == 0:
            cp_wqa(*wg[0], 0).wait()
        for cpy in (queue.pop(0) if queue else []):
            cpy.start()
        with scope("p1_rows"):
            qp_a(*xr[i], *wg[0])
    for item in queue:
        for cpy in item:
            cpy.start()
    for i in range(1, len(wg)):
        cp_wqa(*wg[i], i).wait()
        pre_stage()
        with scope("p1_main"):
            h0, nh = wg[i]
            for a in range(h0, h0 + nh, 4):
                qp_a(0, M, a, min(4, h0 + nh - a))
    while stages:
        pre_stage()
    wait(kb.at[0], ksem.at[0])
    cp_x(1, 0, M, len(xr)).wait()
    s_scr[0] = QK(0, 0, 0)

    def out_copy(br, r0, n, i):
        return pltpu.make_async_copy(ob.at[br, pl.ds(r0, n)], out.at[pl.ds(r0, n), pl.ds(br * D, D)], osem.at[i])

    def chunk_body(br, c, slot, do_qp, last=False):
        g = br * NC + c
        nslot = jnp.where(slot == NS - 1, 0, slot + 1)
        gp = jnp.maximum(g - 1, 0)
        pbr = 0 if br == 0 else jnp.where(c == 0, 0, 1)
        if not last:
            wait(kb.at[nslot], ksem.at[nslot])
        wait(vb.at[slot], vsem.at[slot])
        wait(wob.at[g], wosem.at[g])
        if do_qp:
            wait(wqb.at[c], wqsem.at[c])
        pend = []
        if last:
            pend.append(out_copy(0, 0, M, B))
            pend[-1].start()
        o = o_scr[...]
        for t in range(U):
            if t + 1 < U:
                s_scr[(t + 1) % 2] = QK(g, t + 1, slot)
            elif not last:
                s_scr[0] = QK(g + 1, 0, nslot)
            if do_qp:
                h, b = t // B, t % B
                qb[NC + c, rows(b), cols(h)] = proj_q(xb[1, rows(b), :], wqb[c, :, cols(h)])
            p, l = SM(s_scr[t % 2])
            o_new = PV(p, l, t, slot)
            if t == 0:
                OP(o, pbr, gp, U - 1)
            else:
                fin = last and t - 1 >= U - B
                OP(o, br, g, t - 1, final=fin)
                if fin:
                    b = (t - 1) % B
                    pend.append(out_copy(1, b * SQ, SQ, b))
                    pend[-1].start()
            o = o_new
        if last:
            OP(o, br, g, U - 1, final=True)
            pend.append(out_copy(1, (B - 1) * SQ, SQ, B - 1))
            pend[-1].start()
            for cpy in pend:
                cpy.wait()
        else:
            o_scr[...] = o

    def loop(br, do_qp):
        def body(c, slot):
            with scope("body%d" % br):
                chunk_body(br, c, slot, do_qp)
                if br == 1:
                    r0 = pl.multiple_of(jnp.minimum(c * RA, M - RA), 16)
                    ob[0, pl.ds(r0, RA), :] = acc[0, pl.ds(r0, RA), :].astype(jnp.bfloat16)
            cn = c + NS
            if br == 0:
                @pl.when(cn < NC)
                def _():
                    start_chunk(0, cn, slot)

                @pl.when(cn >= NC)
                def _():
                    start_chunk(1, cn - NC, slot)
            else:
                @pl.when(cn < NC)
                def _():
                    start_chunk(1, cn, slot)
            return jnp.where(slot == NS - 1, 0, slot + 1)
        return body

    slot = jax.lax.fori_loop(0, NC, loop(0, True), jnp.int32(0))
    slot = jax.lax.fori_loop(0, NC - 1, loop(1, False), slot)
    with scope("final"):
        chunk_body(1, NC - 1, slot, False, last=True)


@jax.jit
def pallas_concat_heads__mha_block_cached__mha_block_cached__near_ridge_kernel(
    A_x, A_k_cache, A_v_cache, A_wq, A_wo, B_x, B_k_cache, B_v_cache, B_wq, B_wo):
    bf, f32 = jnp.bfloat16, jnp.float32
    DMA = pltpu.SemaphoreType.DMA
    out = pl.pallas_call(
        _kernel,
        in_specs=[pl.BlockSpec(memory_space=pl.ANY)] * 10,
        out_specs=pl.BlockSpec(memory_space=pl.ANY),
        out_shape=jax.ShapeDtypeStruct((M, 2 * D), bf),
        scratch_shapes=[
            pltpu.VMEM((2, M, D), bf),
            pltpu.VMEM((NS, B, G, SK, DH), bf),
            pltpu.VMEM((NS, B, G, SK, DH), bf),
            pltpu.VMEM((D, H * DH), bf),
            pltpu.VMEM((NC, D, GW), bf),
            pltpu.VMEM((2 * NC, GW, D), bf),
            pltpu.VMEM((2 * NC, M, GW), bf),
            pltpu.VMEM((2, M, D), f32),
            pltpu.VMEM((2, M, D), bf),
            pltpu.VMEM((2, SQ, SK), f32),
            pltpu.VMEM((SQ, DH), bf),
            DMA((len(XR) + 1,)), DMA((NS,)), DMA((NS,)), DMA((8,)), DMA((NC,)), DMA((2 * NC,)), DMA((B + 1,)),
        ],
        compiler_params=pltpu.CompilerParams(vmem_limit_bytes=120 * 1024 * 1024, disable_bounds_checks=True),
    )(A_x.reshape(M, D), A_k_cache, A_v_cache, A_wq, A_wo,
      B_x.reshape(M, D), B_k_cache, B_v_cache, B_wq, B_wo)
    return out.reshape(B, SQ, 2 * D)
```

```python
import contextlib
import os
import jax
import jax.numpy as jnp
import numpy as np
import jax.experimental.pallas as pl
import jax.experimental.pallas.tpu as pltpu

B, SQ, D = 8, 160, 512
H, SK, DH = 32, 512, 128
M = B * SQ
QSCALE = float(DH ** -0.5) * float(np.log2(np.e))

def _env(n, d):
    return os.environ.get(n, d)

G = int(_env("G", 4))
NS = int(_env("NS", 4))
U = G * B
NC = H // G
GW = G * DH
RA = -(-M // ((NC // int(_env('CPB', 1)) - 1) * 16)) * 16
XR = [int(v) for v in _env("XR", "1,2,2,3").split(",")]
WG = [int(v) for v in _env("WG", "4,4,24").split(",")]
PRESTAGE = [int(float(v) * 2**20) for v in _env("PRESTAGE", "200").split(",")]
NOSEMCHK = bool(int(_env("NOSEMCHK", 1)))
QPFIRST = bool(int(_env("QPFIRST", 1)))
CPB = int(_env("CPB", 1))
PREQK = bool(int(_env("PREQK", 0)))
SCOPES = [v for v in _env("SCOPES", "").split(",") if v]
scope = lambda n: jax.named_scope(n) if (n in SCOPES or "1" in SCOPES) else contextlib.nullcontext()


def _kernel(ax, ak, av, awq, awo, bx, bk, bv, bwq, bwo, out,
            xb, kb, vb, wqa, wqb, wob, qb, acc, ob, s_scr, o_scr,
            xsem, ksem, vsem, wqasem, wqsem, wosem, osem):
    xs, ks, vs, wos = (ax, bx), (ak, bk), (av, bv), (awo, bwo)

    def cp_x(br, r0, n, i):
        return pltpu.make_async_copy(xs[br].at[pl.ds(r0, n)], xb.at[br, pl.ds(r0, n)], xsem.at[i])

    def cp_k(br, c, slot):
        return pltpu.make_async_copy(ks[br].at[:, pl.ds(c * G, G)], kb.at[slot], ksem.at[slot])

    def cp_v(br, c, slot):
        return pltpu.make_async_copy(vs[br].at[:, pl.ds(c * G, G)], vb.at[slot], vsem.at[slot])

    def cp_wqa(h0, nh, i):
        return pltpu.make_async_copy(awq.at[:, h0 * DH:(h0 + nh) * DH], wqa.at[:, h0 * DH:(h0 + nh) * DH], wqasem.at[i])

    def cp_wq(c, slot):
        return pltpu.make_async_copy(bwq.at[:, pl.ds(pl.multiple_of(c * GW, GW), GW)], wqb.at[c], wqsem.at[slot])

    def cp_wo(br, c, slot):
        return pltpu.make_async_copy(wos[br].at[pl.ds(pl.multiple_of(c * GW, GW), GW), :],
                                     wob.at[br * NC + c], wosem.at[slot])

    def start_chunk(br, c, slot):
        cp_k(br, c, slot).start()
        cp_v(br, c, slot).start()
        cp_wo(br, c, slot).start()
        if br == 0:
            cp_wq(c, slot).start()

    def wait(dst, sem):
        pltpu.make_async_copy(dst, dst, sem).wait()

    def rows(b):
        return slice(b * SQ, (b + 1) * SQ)

    def cols(h):
        return slice(h * DH, (h + 1) * DH)

    def proj_q(x, w):
        r = jnp.dot(x, w, preferred_element_type=jnp.float32)
        return (r * QSCALE).astype(jnp.bfloat16)

    def QK(g, t, slot):
        h, b = t // B, t % B
        return jax.lax.dot_general(qb[g, rows(b), cols(h)], kb[slot, b, h], (((1,), (1,)), ((), ())),
                                   preferred_element_type=jnp.float32)

    def SM(s):
        m = jnp.max(s, axis=-1, keepdims=True)
        e = jnp.exp2(s - m)
        return e.astype(jnp.bfloat16), jnp.sum(e, axis=-1, keepdims=True)

    def PV(p, l, t, slot):
        h, b = t // B, t % B
        r = jnp.dot(p, vb[slot, b, h], preferred_element_type=jnp.float32)
        return (r * pltpu.reciprocal(l, approx=False, full_range=False)).astype(jnp.bfloat16)

    def OP(o, br, g, t, final=False):
        h, b = t // B, t % B
        r = acc[br, rows(b), :] + jnp.dot(o, wob[g, cols(h), :], preferred_element_type=jnp.float32)
        if final:
            ob[1, rows(b), :] = r.astype(jnp.bfloat16)
        else:
            acc[br, rows(b), :] = r

    xr, wg = [], []
    for n in XR:
        xr.append((sum(v[1] for v in xr), n * SQ))
    for n in WG:
        wg.append((sum(v[1] for v in wg), n))

    def qp_a(r0, n, h0, nh):
        r = proj_q(xb[0, r0:r0 + n, :], wqa[:, h0 * DH:(h0 + nh) * DH])
        for h in range(h0, h0 + nh):
            qb[h // G, r0:r0 + n, cols(h % G)] = r[:, cols(h - h0)]

    KVB, WB, XB = B * G * SK * DH * 2, D * GW * 2, M * D * 2
    pre = [(cp_k(0, 0, 0), KVB), (cp_v(0, 0, 0), KVB), (cp_wo(0, 0, 0), WB), (cp_wq(0, 0), WB), (cp_x(1, 0, M, len(xr)), XB)]
    for g in range(1, NS):
        pre += [(cp_k(0, g, g), KVB), (cp_v(0, g, g), KVB), (cp_wo(0, g, g), WB), (cp_wq(g, g), WB)]
    stages, cur, lim = [[]], 0, list(PRESTAGE)
    for cpy, nb in pre:
        if lim and cur >= lim[0]:
            stages.append([]); cur = 0; lim.pop(0)
        stages[-1].append(cpy); cur += nb

    def pre_stage():
        if stages:
            for cpy in stages.pop(0):
                cpy.start()

    cp_x(0, *xr[0], 0).start()
    cp_wqa(*wg[0], 0).start()
    cp_x(0, *xr[1], 1).start()
    acc[...] = jnp.zeros_like(acc)
    o_scr[...] = jnp.zeros_like(o_scr)
    queue = [[cp_x(0, *xr[i], i)] for i in range(2, len(xr))]
    queue += [[cp_wqa(*wg[1], 1)], [cp_wqa(*wg[i], i) for i in range(2, len(wg))]]
    for i in range(len(xr)):
        cp_x(0, *xr[i], i).wait()
        if i == 0:
            cp_wqa(*wg[0], 0).wait()
        for cpy in (queue.pop(0) if queue else []):
            cpy.start()
        with scope("p1_rows"):
            qp_a(*xr[i], *wg[0])
    for item in queue:
        for cpy in item:
            cpy.start()
    for i in range(1, len(wg)):
        cp_wqa(*wg[i], i).wait()
        lastblk = PREQK and i == len(wg) - 1
        if lastblk:
            wait(kb.at[0], ksem.at[0])
        pre_stage()
        with scope("p1_main"):
            h0, nh = wg[i]
            for a in range(h0, h0 + nh, 4):
                qp_a(0, M, a, min(4, h0 + nh - a))
            if lastblk:
                s_scr[0] = QK(0, 0, 0)
    while stages:
        pre_stage()
    cp_x(1, 0, M, len(xr)).wait()
    if not PREQK:
        wait(kb.at[0], ksem.at[0])
        s_scr[0] = QK(0, 0, 0)

    def out_copy(br, r0, n, i):
        return pltpu.make_async_copy(ob.at[br, pl.ds(r0, n)], out.at[pl.ds(r0, n), pl.ds(br * D, D)], osem.at[0])

    def nxt(slot):
        return jnp.where(slot == NS - 1, 0, slot + 1)

    def chunk_waits(br, c, slot, do_qp, last=False):
        if not last:
            wait(kb.at[nxt(slot)], ksem.at[nxt(slot)])
        wait(vb.at[slot], vsem.at[slot])
        wait(wob.at[br * NC + c], wosem.at[slot])
        if do_qp:
            wait(wqb.at[c], wqsem.at[slot])

    def chunk_body(br, c, slot, do_qp, last=False):
        g = br * NC + c
        nslot = nxt(slot)
        gp = jnp.maximum(g - 1, 0)
        pbr = 0 if br == 0 else jnp.where(c == 0, 0, 1)
        pend = []
        o = o_scr[...]
        for t in range(U):
            def do_qk():
                if t + 1 < U:
                    s_scr[(t + 1) % 2] = QK(g, t + 1, slot)
                elif not last:
                    s_scr[0] = QK(g + 1, 0, nslot)

            def do_qp_():
                if do_qp:
                    h, b = t // B, t % B
                    qb[NC + c, rows(b), cols(h)] = proj_q(xb[1, rows(b), :], wqb[c, :, cols(h)])

            if QPFIRST:
                do_qp_(); do_qk()
            else:
                do_qk(); do_qp_()
            p, l = SM(s_scr[t % 2])
            o_new = PV(p, l, t, slot)
            if t == 0:
                OP(o, pbr, gp, U - 1)
            else:
                fin = last and t - 1 >= U - B
                OP(o, br, g, t - 1, final=fin)
                if fin:
                    b = (t - 1) % B
                    pend.append(out_copy(1, b * SQ, SQ, b))
                    pend[-1].start()
            o = o_new
        if last:
            OP(o, br, g, U - 1, final=True)
            pend.append(out_copy(1, (B - 1) * SQ, SQ, B - 1))
            pend[-1].start()
            for cpy in pend:
                cpy.wait()
        else:
            o_scr[...] = o

    def refill(br, c, slot):
        cn = c + NS
        if br == 0:
            @pl.when(cn < NC)
            def _():
                start_chunk(0, cn, slot)

            @pl.when(cn >= NC)
            def _():
                start_chunk(1, cn - NC, slot)
        else:
            @pl.when(cn < NC)
            def _():
                start_chunk(1, cn, slot)

    def loop(br, do_qp):
        def body(j, slot):
            with scope("body%d" % br):
                slots = [slot]
                for i in range(1, CPB):
                    slots.append(nxt(slots[-1]))
                for i in range(CPB):
                    chunk_waits(br, j * CPB + i, slots[i], do_qp)
                if br == 1:
                    r0 = pl.multiple_of(jnp.minimum(j * RA, M - RA), 16)
                    ob[0, pl.ds(r0, RA), :] = acc[0, pl.ds(r0, RA), :].astype(jnp.bfloat16)
                for i in range(CPB):
                    chunk_body(br, j * CPB + i, slots[i], do_qp)
                    refill(br, j * CPB + i, slots[i])
            return nxt(slots[-1])
        return body

    slot = jax.lax.fori_loop(0, NC // CPB, loop(0, True), jnp.int32(0))
    slot = jax.lax.fori_loop(0, NC // CPB - 1, loop(1, False), slot)
    with scope("final"):
        slots = [slot]
        for i in range(1, CPB):
            slots.append(nxt(slots[-1]))
        for i in range(CPB):
            chunk_waits(1, NC - CPB + i, slots[i], False, last=(i == CPB - 1))
        aout = out_copy(0, 0, M, B)
        aout.start()
        for i in range(CPB):
            chunk_body(1, NC - CPB + i, slots[i], False, last=(i == CPB - 1))
        aout.wait()


@jax.jit
def pallas_concat_heads__mha_block_cached__mha_block_cached__near_ridge_kernel(
    A_x, A_k_cache, A_v_cache, A_wq, A_wo, B_x, B_k_cache, B_v_cache, B_wq, B_wo):
    bf, f32 = jnp.bfloat16, jnp.float32
    DMA = pltpu.SemaphoreType.DMA
    out = pl.pallas_call(
        _kernel,
        in_specs=[pl.BlockSpec(memory_space=pl.ANY)] * 10,
        out_specs=pl.BlockSpec(memory_space=pl.ANY),
        out_shape=jax.ShapeDtypeStruct((M, 2 * D), bf),
        scratch_shapes=[
            pltpu.VMEM((2, M, D), bf),
            pltpu.VMEM((NS, B, G, SK, DH), bf),
            pltpu.VMEM((NS, B, G, SK, DH), bf),
            pltpu.VMEM((D, H * DH), bf),
            pltpu.VMEM((NC, D, GW), bf),
            pltpu.VMEM((2 * NC, GW, D), bf),
            pltpu.VMEM((2 * NC, M, GW), bf),
            pltpu.VMEM((2, M, D), f32),
            pltpu.VMEM((2, M, D), bf),
            pltpu.VMEM((2, SQ, SK), f32),
            pltpu.VMEM((SQ, DH), bf),
            DMA((len(XR) + 1,)), DMA((NS,)), DMA((NS,)), DMA((len(WG),)), DMA((NS,)), DMA((NS,)), DMA((1,)),
        ],
        compiler_params=pltpu.CompilerParams(vmem_limit_bytes=120 * 1024 * 1024, disable_bounds_checks=True, disable_semaphore_checks=NOSEMCHK),
    )(A_x.reshape(M, D), A_k_cache, A_v_cache, A_wq, A_wo,
      B_x.reshape(M, D), B_k_cache, B_v_cache, B_wq, B_wo)
    return out.reshape(B, SQ, 2 * D)
```

```python
import jax
import jax.numpy as jnp
import numpy as np
import jax.experimental.pallas as pl
import jax.experimental.pallas.tpu as pltpu

B, SQ, D = 8, 160, 512
H, SK, DH = 32, 512, 128
M = B * SQ

G = 4
U = G * B
NC = H // G
GW = G * DH
NS = 4

QSCALE = float(DH ** -0.5) * float(np.log2(np.e))

WQ_PIECES = ((0, 1), (1, 1), (2, 1), (3, 1), (4, 4), (8, 8), (16, 16))
LOOP_HEADS = 8
ZERO_ROWS = 80
A_ROWS = -(-M // ((NC - 1) * 16)) * 16


def _kernel(ax, ak, av, awq, awo, bx, bk, bv, bwq, bwo, out,
            xb, kb, vb, wqa, wqb, wob, qb, acc, ob, s_scr, o_scr,
            xsem, ksem, vsem, wqasem, wqsem, wosem, osem):
    xs, ks, vs, wos = (ax, bx), (ak, bk), (av, bv), (awo, bwo)

    def cp_x(br, r0, n, i):
        return pltpu.make_async_copy(xs[br].at[pl.ds(r0, n)], xb.at[br, pl.ds(r0, n)], xsem.at[i])

    def cp_k(br, c, slot):
        return pltpu.make_async_copy(ks[br].at[:, pl.ds(c * G, G)], kb.at[slot], ksem.at[slot])

    def cp_v(br, c, slot):
        return pltpu.make_async_copy(vs[br].at[:, pl.ds(c * G, G)], vb.at[slot], vsem.at[slot])

    def cp_wqa(h0, nh, i):
        return pltpu.make_async_copy(awq.at[:, h0 * DH:(h0 + nh) * DH],
                                     wqa.at[:, h0 * DH:(h0 + nh) * DH], wqasem.at[i])

    def cp_wqb(c, slot):
        return pltpu.make_async_copy(bwq.at[:, pl.ds(pl.multiple_of(c * GW, GW), GW)],
                                     wqb.at[c], wqsem.at[slot])

    def cp_wo(br, c, slot):
        return pltpu.make_async_copy(wos[br].at[pl.ds(pl.multiple_of(c * GW, GW), GW), :],
                                     wob.at[br * NC + c], wosem.at[slot])

    def cp_out(br, r0, n):
        return pltpu.make_async_copy(ob.at[br, pl.ds(r0, n)],
                                     out.at[pl.ds(r0, n), pl.ds(br * D, D)], osem.at[0])

    def chunk_copies(br, c, slot):
        cps = [cp_k(br, c, slot), cp_v(br, c, slot), cp_wo(br, c, slot)]
        return cps + [cp_wqb(c, slot)] if br == 0 else cps

    def wait(dst, sem):
        pltpu.make_async_copy(dst, dst, sem).wait()

    def rows(b):
        return slice(b * SQ, (b + 1) * SQ)

    def cols(h):
        return slice(h * DH, (h + 1) * DH)

    def proj_q(x, w):
        r = jnp.dot(x, w, preferred_element_type=jnp.float32)
        return (r * QSCALE).astype(jnp.bfloat16)

    def stage_qk(g, t, slot):
        h, b = t // B, t % B
        return jax.lax.dot_general(qb[g * G + h, rows(b), :], kb[slot, b, h],
                                   (((1,), (1,)), ((), ())), preferred_element_type=jnp.float32)

    def stage_softmax_pv(s, t, slot):
        h, b = t // B, t % B
        m = jnp.max(s, axis=-1, keepdims=True)
        e = jnp.exp2(s - m)
        l = jnp.sum(e, axis=-1, keepdims=True)
        r = jnp.dot(e.astype(jnp.bfloat16), vb[slot, b, h], preferred_element_type=jnp.float32)
        return (r * pltpu.reciprocal(l, approx=False, full_range=False)).astype(jnp.bfloat16)

    def stage_op(o, br, g, t, final=False):
        h, b = t // B, t % B
        r = acc[br, rows(b), :] + jnp.dot(o, wob[g, cols(h), :], preferred_element_type=jnp.float32)
        if final:
            ob[br, rows(b), :] = r.astype(jnp.bfloat16)
        else:
            acc[br, rows(b), :] = r

    def qp_a(r0, n, h0, nh):
        r = proj_q(xb[0, r0:r0 + n, :], wqa[:, h0 * DH:(h0 + nh) * DH])
        for h in range(nh):
            qb[h0 + h, r0:r0 + n, :] = r[:, cols(h)]

    xp = [cp_x(0, b * SQ, SQ, b) for b in range(B)]
    wp = [cp_wqa(h0, nh, i) for i, (h0, nh) in enumerate(WQ_PIECES)]
    x_b = cp_x(1, 0, M, B)
    groups = [[xp[0], wp[0]], [xp[1], wp[1]], [xp[2], wp[2]], [xp[3], wp[3]], xp[4:6], xp[6:8]]
    grow = ((1, 1), (1, 1), (1, 1), (1, 1), (2, 0), (2, 0))
    groups += [[w] for w in wp[4:]]
    groups += [[x_b] + chunk_copies(0, 0, 0)] + [chunk_copies(0, g, g) for g in range(1, NS)]

    zpb = SQ // ZERO_ROWS
    nz = 2 * B * zpb
    z0 = 0
    for gi, grp in enumerate(groups):
        for cpy in grp:
            cpy.start()
        z1 = (gi + 1) * nz // len(groups)

        def zero(i, carry):
            r0 = pl.multiple_of((i % (B * zpb)) * ZERO_ROWS, 8)
            acc[i // (B * zpb), pl.ds(r0, ZERO_ROWS), :] = jnp.zeros((ZERO_ROWS, D), jnp.float32)
            return carry

        jax.lax.fori_loop(z0, z1, zero, 0)
        z0 = z1
    o_scr[...] = jnp.zeros_like(o_scr)

    nb = nh = 0
    for grp, (db, dh) in zip(groups, grow):
        for cpy in grp:
            cpy.wait()
        if dh:
            if nb:
                qp_a(0, nb * SQ, nh, dh)
            nh += dh
        qp_a(nb * SQ, db * SQ, 0, nh)
        nb += db
    for w, (h0, n) in list(zip(wp, WQ_PIECES))[4:]:
        w.wait()
        if n >= 2 * LOOP_HEADS:
            def qp_loop(i, carry, h0=h0):
                for a in range(0, LOOP_HEADS, G):
                    hh = h0 + i * LOOP_HEADS + a
                    r = proj_q(xb[0], wqa[:, pl.ds(pl.multiple_of(hh * DH, DH), GW)])
                    for h in range(G):
                        qb[hh + h] = r[:, cols(h)]
                return carry

            jax.lax.fori_loop(0, n // LOOP_HEADS, qp_loop, 0)
        else:
            for a in range(h0, h0 + n, G):
                qp_a(0, M, a, min(G, h0 + n - a))
    x_b.wait()
    wait(kb.at[0], ksem.at[0])
    s_scr[0] = stage_qk(0, 0, 0)

    def next_slot(slot):
        return jnp.where(slot == NS - 1, 0, slot + 1)

    def chunk(br, c, slot, last=False):
        g = br * NC + c
        nslot = next_slot(slot)
        gp = jnp.maximum(g - 1, 0)
        pbr = 0 if br == 0 else (1 if last else jnp.where(c == 0, 0, 1))
        wait(vb.at[slot], vsem.at[slot])
        wait(wob.at[g], wosem.at[slot])
        if br == 0:
            wait(wqb.at[c], wqsem.at[slot])
        pending = []
        if last:
            pending.append(cp_out(0, 0, M))
            pending[-1].start()
        elif br == 1:
            r0 = pl.multiple_of(jnp.minimum(c * A_ROWS, M - A_ROWS), 16)
            ob[0, pl.ds(r0, A_ROWS), :] = acc[0, pl.ds(r0, A_ROWS), :].astype(jnp.bfloat16)
        o = o_scr[...]
        for t in range(U):
            h, b = t // B, t % B
            if br == 0:
                qb[H + c * G + h, rows(b), :] = proj_q(xb[1, rows(b), :], wqb[c, :, cols(h)])
            if t + 1 < U:
                s_scr[(t + 1) % 2] = stage_qk(g, t + 1, slot)
            elif not last:
                wait(kb.at[nslot], ksem.at[nslot])
                s_scr[0] = stage_qk(g + 1, 0, nslot)
            o_new = stage_softmax_pv(s_scr[t % 2], t, slot)
            if t == 0:
                stage_op(o, pbr, gp, U - 1)
            else:
                fin = last and t - 1 >= U - B
                stage_op(o, br, g, t - 1, final=fin)
                if fin:
                    pending.append(cp_out(1, ((t - 1) % B) * SQ, SQ))
                    pending[-1].start()
            o = o_new
        if last:
            stage_op(o, br, g, U - 1, final=True)
            pending.append(cp_out(1, (B - 1) * SQ, SQ))
            pending[-1].start()
            for cpy in pending:
                cpy.wait()
        else:
            o_scr[...] = o

    def chunk_loop(br):
        def body(c, slot):
            chunk(br, c, slot)
            cn = c + NS

            def refill(src_br, src_c):
                for cpy in chunk_copies(src_br, src_c, slot):
                    cpy.start()

            pl.when(cn < NC)(lambda: refill(br, cn))
            if br == 0:
                pl.when(cn >= NC)(lambda: refill(1, cn - NC))
            return next_slot(slot)

        return body

    slot = jax.lax.fori_loop(0, NC, chunk_loop(0), jnp.int32(0))
    slot = jax.lax.fori_loop(0, NC - 1, chunk_loop(1), slot)
    chunk(1, NC - 1, slot, last=True)


@jax.jit
def pallas_concat_heads__mha_block_cached__mha_block_cached__near_ridge_kernel(
    A_x: jax.Array,
    A_k_cache: jax.Array,
    A_v_cache: jax.Array,
    A_wq: jax.Array,
    A_wo: jax.Array,
    B_x: jax.Array,
    B_k_cache: jax.Array,
    B_v_cache: jax.Array,
    B_wq: jax.Array,
    B_wo: jax.Array,
):
    bf16, f32 = jnp.bfloat16, jnp.float32
    dma = pltpu.SemaphoreType.DMA
    out = pl.pallas_call(
        _kernel,
        in_specs=[pl.BlockSpec(memory_space=pl.ANY)] * 10,
        out_specs=pl.BlockSpec(memory_space=pl.ANY),
        out_shape=jax.ShapeDtypeStruct((M, 2 * D), bf16),
        scratch_shapes=[
            pltpu.VMEM((2, M, D), bf16),
            pltpu.VMEM((NS, B, G, SK, DH), bf16),
            pltpu.VMEM((NS, B, G, SK, DH), bf16),
            pltpu.VMEM((D, H * DH), bf16),
            pltpu.VMEM((NC, D, GW), bf16),
            pltpu.VMEM((2 * NC, GW, D), bf16),
            pltpu.VMEM((2 * H, M, DH), bf16),
            pltpu.VMEM((2, M, D), f32),
            pltpu.VMEM((2, M, D), bf16),
            pltpu.VMEM((2, SQ, SK), f32),
            pltpu.VMEM((SQ, DH), bf16),
            dma((B + 1,)), dma((NS,)), dma((NS,)), dma((len(WQ_PIECES),)),
            dma((NS,)), dma((NS,)), dma((1,)),
        ],
        compiler_params=pltpu.CompilerParams(
            vmem_limit_bytes=120 * 1024 * 1024,
            disable_bounds_checks=True,
            disable_semaphore_checks=True,
            flags={"XLA_TPU_RESCHEDULE_DMA_DONES": True},
        ),
    )(A_x.reshape(M, D), A_k_cache, A_v_cache, A_wq, A_wo,
      B_x.reshape(M, D), B_k_cache, B_v_cache, B_wq, B_wo)
    return out.reshape(B, SQ, 2 * D)
```

```python
import jax
import jax.numpy as jnp
import numpy as np
import jax.experimental.pallas as pl
import jax.experimental.pallas.tpu as pltpu

B, SQ, D = 8, 160, 512
H, SK, DH = 32, 512, 128
M = B * SQ

G = 4
U = G * B
NC = H // G
GW = G * DH
NS = 4

QSCALE = float(DH ** -0.5) * float(np.log2(np.e))

WQ_PIECES = ((0, 1), (1, 1), (2, 1), (3, 1), (4, 4), (8, 8), (16, 16))
LOOP_HEADS = 8
ZERO_ROWS = 80
A_ROWS = -(-M // ((NC - 1) * 16)) * 16


def _kernel(ax, ak, av, awq, awo, bx, bk, bv, bwq, bwo, out,
            xb, kb, vb, wqa, wqb, wob, qb, acc, ob, s_scr, o_scr,
            xsem, ksem, vsem, wqasem, wqsem, wosem, osem):
    xs, ks, vs, wos = (ax, bx), (ak, bk), (av, bv), (awo, bwo)

    def cp_x(br, r0, n, i):
        return pltpu.make_async_copy(xs[br].at[pl.ds(r0, n)], xb.at[br, pl.ds(r0, n)], xsem.at[i])

    def cp_k(br, c, slot):
        return pltpu.make_async_copy(ks[br].at[:, pl.ds(c * G, G)], kb.at[slot], ksem.at[slot])

    def cp_v(br, c, slot):
        return pltpu.make_async_copy(vs[br].at[:, pl.ds(c * G, G)], vb.at[slot], vsem.at[slot])

    def cp_wqa(h0, nh, i):
        return pltpu.make_async_copy(awq.at[:, h0 * DH:(h0 + nh) * DH],
                                     wqa.at[:, h0 * DH:(h0 + nh) * DH], wqasem.at[i])

    def cp_wqb(c, slot):
        return pltpu.make_async_copy(bwq.at[:, pl.ds(pl.multiple_of(c * GW, GW), GW)],
                                     wqb.at[c], wqsem.at[slot])

    def cp_wo(br, c, slot):
        return pltpu.make_async_copy(wos[br].at[pl.ds(pl.multiple_of(c * GW, GW), GW), :],
                                     wob.at[br * NC + c], wosem.at[slot])

    def cp_out(br, r0, n):
        return pltpu.make_async_copy(ob.at[br, pl.ds(r0, n)],
                                     out.at[pl.ds(r0, n), pl.ds(br * D, D)], osem.at[0])

    def chunk_copies(br, c, slot):
        cps = [cp_k(br, c, slot), cp_v(br, c, slot), cp_wo(br, c, slot)]
        return cps + [cp_wqb(c, slot)] if br == 0 else cps

    def wait(dst, sem):
        pltpu.make_async_copy(dst, dst, sem).wait()

    def rows(b):
        return slice(b * SQ, (b + 1) * SQ)

    def cols(h):
        return slice(h * DH, (h + 1) * DH)

    def proj_q(x, w):
        r = jnp.dot(x, w, preferred_element_type=jnp.float32)
        return (r * QSCALE).astype(jnp.bfloat16)

    def stage_qk(g, t, slot):
        h, b = t // B, t % B
        return jax.lax.dot_general(qb[g * G + h, rows(b), :], kb[slot, b, h],
                                   (((1,), (1,)), ((), ())), preferred_element_type=jnp.float32)

    def stage_softmax_pv(s, t, slot):
        h, b = t // B, t % B
        m = jnp.max(s, axis=-1, keepdims=True)
        e = jnp.exp2(s - m)
        l = jnp.sum(e, axis=-1, keepdims=True)
        r = jnp.dot(e.astype(jnp.bfloat16), vb[slot, b, h], preferred_element_type=jnp.float32)
        return (r * pltpu.reciprocal(l, approx=False, full_range=False)).astype(jnp.bfloat16)

    def stage_op(o, br, g, t, final=False):
        h, b = t // B, t % B
        r = acc[br, rows(b), :] + jnp.dot(o, wob[g, cols(h), :], preferred_element_type=jnp.float32)
        if final:
            ob[br, rows(b), :] = r.astype(jnp.bfloat16)
        else:
            acc[br, rows(b), :] = r

    def qp_a(r0, n, h0, nh):
        r = proj_q(xb[0, r0:r0 + n, :], wqa[:, h0 * DH:(h0 + nh) * DH])
        for h in range(nh):
            qb[h0 + h, r0:r0 + n, :] = r[:, cols(h)]

    xp = [cp_x(0, b * SQ, SQ, b) for b in range(B)]
    wp = [cp_wqa(h0, nh, i) for i, (h0, nh) in enumerate(WQ_PIECES)]
    x_b = cp_x(1, 0, M, B)
    groups = [[xp[0], wp[0]], [xp[1]], [wp[1]], [xp[2]], [wp[2]], [xp[3]], [wp[3]], xp[4:6], xp[6:8]]
    grow = ((1, 1), (1, 0), (0, 1), (1, 0), (0, 1), (1, 0), (0, 1), (2, 0), (2, 0))
    groups += [[w] for w in wp[4:]]
    groups += [[x_b] + chunk_copies(0, 0, 0)] + [chunk_copies(0, g, g) for g in range(1, NS)]

    zpb = SQ // ZERO_ROWS
    nz = 2 * B * zpb
    z0 = 0
    for gi, grp in enumerate(groups):
        for cpy in grp:
            cpy.start()
        z1 = (gi + 1) * nz // len(groups)

        def zero(i, carry):
            r0 = pl.multiple_of((i % (B * zpb)) * ZERO_ROWS, 8)
            acc[i // (B * zpb), pl.ds(r0, ZERO_ROWS), :] = jnp.zeros((ZERO_ROWS, D), jnp.float32)
            return carry

        jax.lax.fori_loop(z0, z1, zero, 0)
        z0 = z1
    o_scr[...] = jnp.zeros_like(o_scr)

    nb = nh = 0
    for grp, (db, dh) in zip(groups, grow):
        for cpy in grp:
            cpy.wait()
        if dh:
            if nb:
                qp_a(0, nb * SQ, nh, dh)
            nh += dh
        if db:
            qp_a(nb * SQ, db * SQ, 0, nh)
            nb += db
    for w, (h0, n) in list(zip(wp, WQ_PIECES))[4:]:
        w.wait()
        if n >= 2 * LOOP_HEADS:
            def qp_loop(i, carry, h0=h0):
                for a in range(0, LOOP_HEADS, G):
                    hh = h0 + i * LOOP_HEADS + a
                    r = proj_q(xb[0], wqa[:, pl.ds(pl.multiple_of(hh * DH, DH), GW)])
                    for h in range(G):
                        qb[hh + h] = r[:, cols(h)]
                return carry

            jax.lax.fori_loop(0, n // LOOP_HEADS, qp_loop, 0)
        else:
            for a in range(h0, h0 + n, G):
                qp_a(0, M, a, min(G, h0 + n - a))
    x_b.wait()
    wait(kb.at[0], ksem.at[0])
    s_scr[0] = stage_qk(0, 0, 0)

    def next_slot(slot):
        return jnp.where(slot == NS - 1, 0, slot + 1)

    def chunk(br, c, slot, last=False):
        g = br * NC + c
        nslot = next_slot(slot)
        gp = jnp.maximum(g - 1, 0)
        pbr = 0 if br == 0 else (1 if last else jnp.where(c == 0, 0, 1))
        wait(vb.at[slot], vsem.at[slot])
        wait(wob.at[g], wosem.at[slot])
        if br == 0:
            wait(wqb.at[c], wqsem.at[slot])
        pending = []
        if last:
            pending.append(cp_out(0, 0, M))
            pending[-1].start()
        elif br == 1:
            r0 = pl.multiple_of(jnp.minimum(c * A_ROWS, M - A_ROWS), 16)
            ob[0, pl.ds(r0, A_ROWS), :] = acc[0, pl.ds(r0, A_ROWS), :].astype(jnp.bfloat16)
        o = o_scr[...]
        for t in range(U):
            h, b = t // B, t % B
            if br == 0:
                qb[H + c * G + h, rows(b), :] = proj_q(xb[1, rows(b), :], wqb[c, :, cols(h)])
            if t + 1 < U:
                s_scr[(t + 1) % 2] = stage_qk(g, t + 1, slot)
            elif not last:
                wait(kb.at[nslot], ksem.at[nslot])
                s_scr[0] = stage_qk(g + 1, 0, nslot)
            o_new = stage_softmax_pv(s_scr[t % 2], t, slot)
            if t == 0:
                stage_op(o, pbr, gp, U - 1)
            else:
                fin = last and t - 1 >= U - B
                stage_op(o, br, g, t - 1, final=fin)
                if fin:
                    pending.append(cp_out(1, ((t - 1) % B) * SQ, SQ))
                    pending[-1].start()
            o = o_new
        if last:
            stage_op(o, br, g, U - 1, final=True)
            pending.append(cp_out(1, (B - 1) * SQ, SQ))
            pending[-1].start()
            for cpy in pending:
                cpy.wait()
        else:
            o_scr[...] = o

    def chunk_loop(br):
        def body(c, slot):
            chunk(br, c, slot)
            cn = c + NS

            def refill(src_br, src_c):
                for cpy in chunk_copies(src_br, src_c, slot):
                    cpy.start()

            pl.when(cn < NC)(lambda: refill(br, cn))
            if br == 0:
                pl.when(cn >= NC)(lambda: refill(1, cn - NC))
            return next_slot(slot)

        return body

    slot = jax.lax.fori_loop(0, NC, chunk_loop(0), jnp.int32(0))
    slot = jax.lax.fori_loop(0, NC - 1, chunk_loop(1), slot)
    chunk(1, NC - 1, slot, last=True)


@jax.jit
def pallas_concat_heads__mha_block_cached__mha_block_cached__near_ridge_kernel(
    A_x: jax.Array,
    A_k_cache: jax.Array,
    A_v_cache: jax.Array,
    A_wq: jax.Array,
    A_wo: jax.Array,
    B_x: jax.Array,
    B_k_cache: jax.Array,
    B_v_cache: jax.Array,
    B_wq: jax.Array,
    B_wo: jax.Array,
):
    bf16, f32 = jnp.bfloat16, jnp.float32
    dma = pltpu.SemaphoreType.DMA
    out = pl.pallas_call(
        _kernel,
        in_specs=[pl.BlockSpec(memory_space=pl.ANY)] * 10,
        out_specs=pl.BlockSpec(memory_space=pl.ANY),
        out_shape=jax.ShapeDtypeStruct((M, 2 * D), bf16),
        scratch_shapes=[
            pltpu.VMEM((2, M, D), bf16),
            pltpu.VMEM((NS, B, G, SK, DH), bf16),
            pltpu.VMEM((NS, B, G, SK, DH), bf16),
            pltpu.VMEM((D, H * DH), bf16),
            pltpu.VMEM((NC, D, GW), bf16),
            pltpu.VMEM((2 * NC, GW, D), bf16),
            pltpu.VMEM((2 * H, M, DH), bf16),
            pltpu.VMEM((2, M, D), f32),
            pltpu.VMEM((2, M, D), bf16),
            pltpu.VMEM((2, SQ, SK), f32),
            pltpu.VMEM((SQ, DH), bf16),
            dma((B + 1,)), dma((NS,)), dma((NS,)), dma((len(WQ_PIECES),)),
            dma((NS,)), dma((NS,)), dma((1,)),
        ],
        compiler_params=pltpu.CompilerParams(
            vmem_limit_bytes=120 * 1024 * 1024,
            disable_bounds_checks=True,
            disable_semaphore_checks=True,
            flags={"XLA_TPU_RESCHEDULE_DMA_DONES": True},
        ),
    )(A_x.reshape(M, D), A_k_cache, A_v_cache, A_wq, A_wo,
      B_x.reshape(M, D), B_k_cache, B_v_cache, B_wq, B_wo)
    return out.reshape(B, SQ, 2 * D)
```
